```python
import jax
import jax.numpy as jnp

def _softmax(x, axis=-1):
    return jax.nn.softmax(x, axis=axis)
def _gelu(x):
    return jax.nn.gelu(x, approximate=True)
def _silu(x):
    return jax.nn.silu(x)
def _sigmoid(x):
    return jax.nn.sigmoid(x)
def _layernorm(x, axis=-1, eps=1e-5):
    m = jnp.mean(x, axis=axis, keepdims=True)
    v = jnp.var(x, axis=axis, keepdims=True)
    return (x - m) / jnp.sqrt(v + eps)
def _scatter_add(tgt, idx, src, axis=0):
    return tgt.at[idx].add(src)
def _segment_sum(src, seg, n):
    return jax.ops.segment_sum(src, seg, n)
class _Rng:
    def __init__(self, key):
        self._k = key
    def _next(self):
        self._k, sub = jax.random.split(self._k)
        return sub
    def normal(self, shape):
        return jax.random.normal(self._next(), shape, dtype=jnp.bfloat16)
    def randint(self, lo, hi, shape):
        return jax.random.randint(self._next(), shape, lo, hi, dtype=jnp.int32)
    def uniform(self, shape, lo=0.0, hi=1.0):
        return jax.random.uniform(self._next(), shape, jnp.bfloat16, lo, hi)
    def permutation(self, n):
        return jax.random.permutation(self._next(), n)


kernel_name = 'standalone__depthwise_separable__vision'

def setup_inputs():
    _rng = _Rng(jax.random.key(int.from_bytes(__import__("os").urandom(4), "little")))
    _w = (lambda a: (lambda t: t.astype(jnp.bfloat16) if jnp.issubdtype(t.dtype, jnp.floating) else t)(jnp.asarray(a)))
    H = W = 384
    C = 384
    k = 1
    return {
        "x": _w((lambda *s: _rng.normal(s) * 0.05)(1, H, W, C)),
        "dw": _w((lambda *s: _rng.normal(s) * 0.05)(k, k, C)),
        "pw": _w((lambda *s: _rng.normal(s) * 0.05)(C, C)),
    }

def reference(x, dw, pw):
    B, H, W, C = x.shape
    k = dw.shape[0]
    pad = k // 2
    xp = jnp.pad(x, ((0,0),(pad,pad),(pad,pad),(0,0)))
    out = jnp.zeros_like(x)
    for i in range(k):
        for j in range(k):
            out = out + xp[:, i:i+H, j:j+W, :] * dw[i, j][None, None, None, :]
    return jnp.einsum('bhwc,cd->bhwd', out, pw)
```

```python
import jax
import jax.numpy as jnp
import jax.experimental.pallas as pl
import jax.experimental.pallas.tpu as pltpu

_CHUNK = 32
_UNITS = 32
_STEPS = 2


@jax.jit
def pallas_standalone__depthwise_separable__vision_kernel(
    x: jax.Array,
    dw: jax.Array,
    pw: jax.Array,
):
    B, H, W, C = x.shape
    assert dw.shape == (1, 1, C) and pw.shape == (C, C)
    rows = B * H * W
    groups = rows // (_UNITS * _CHUNK)
    assert groups * _UNITS * _CHUNK == rows and groups % _STEPS == 0
    step_groups = groups // _STEPS
    first = _UNITS // 2

    def kernel_function(x_hbm, dw_ref, pw_ref, o_hbm, buf, read_sems, write_sem):
        def read(u):
            return pltpu.make_async_copy(x_hbm.at[:, u], buf.at[:, u], read_sems.at[u])

        def read_rest():
            rest = pl.ds(first, _UNITS - first)
            return pltpu.make_async_copy(
                x_hbm.at[:, rest], buf.at[:, rest], read_sems.at[first])

        def write(u):
            return pltpu.make_async_copy(buf.at[:, u], o_hbm.at[:, u], write_sem)

        def compute(u):
            @pl.loop(0, _STEPS)
            def _(s):
                g = pl.ds(s * step_groups, step_groups)
                xv = buf[g, u].reshape(step_groups * _CHUNK, C)
                t = xv.astype(jnp.float32) * dw_ref[0].astype(jnp.float32)
                y = jnp.dot(t.astype(xv.dtype), pw_ref[...],
                            preferred_element_type=jnp.float32)
                buf[g, u] = y.astype(buf.dtype).reshape(step_groups, _CHUNK, C)

        @pl.loop(0, first)
        def _(u):
            read(u).start()

        read_rest().start()

        @pl.loop(0, _UNITS)
        def _(u):
            @pl.when(u < first)
            def _():
                read(u).wait()

            @pl.when(u == first)
            def _():
                read_rest().wait()

                @pl.loop(0, first)
                def _(v):
                    write(v).start()

            compute(u)

            @pl.when(u >= first)
            def _():
                write(u).start()

        pltpu.make_async_copy(buf, o_hbm, write_sem).wait()

    view = (groups, _UNITS, _CHUNK, C)
    out = pl.pallas_call(
        kernel_function,
        in_specs=[
            pl.BlockSpec(memory_space=pl.ANY),
            pl.BlockSpec(memory_space=pltpu.VMEM),
            pl.BlockSpec(memory_space=pltpu.VMEM),
        ],
        out_specs=pl.BlockSpec(memory_space=pl.ANY),
        out_shape=jax.ShapeDtypeStruct(view, x.dtype),
        scratch_shapes=[
            pltpu.VMEM(view, x.dtype),
            pltpu.SemaphoreType.DMA((first + 1,)),
            pltpu.SemaphoreType.DMA,
        ],
        compiler_params=pltpu.CompilerParams(vmem_limit_bytes=124 * 1024 * 1024),
    )(x.reshape(view), dw, pw)
    return out.reshape(B, H, W, C)
```

```python
import jax
import jax.numpy as jnp
import jax.experimental.pallas as pl
import jax.experimental.pallas.tpu as pltpu

_STREAMS = 6
_CHUNKS = 128
_CHUNK_ROWS = 32
_STEP = 32
_VMEM_LIMIT = 124 * 1024 * 1024


def _kernel(x_hbm, dw_hbm, pw_hbm, o_hbm,
            buf, dw_ref, pw_ref, step_sems, misc_sems, write_sem):
    blocks, streams, chunks, chunk_rows, C = buf.shape
    steps_per_block = chunks // _STEP
    steps = blocks * steps_per_block
    early_blocks = blocks // 2
    early_steps = early_blocks * steps_per_block

    def step_index(u):
        return (u // steps_per_block, slice(None),
                pl.ds((u % steps_per_block) * _STEP, _STEP))

    def read(index, sem):
        return pltpu.make_async_copy(x_hbm.at[index], buf.at[index], sem)

    def start_writes(first, last):
        @pl.loop(first, last)
        def _(i):
            index = (i // chunks, slice(None), i % chunks)
            pltpu.make_async_copy(buf.at[index], o_hbm.at[index], write_sem).start()

    late = (pl.ds(early_blocks, blocks - early_blocks), slice(None))
    read_late = read(late + (pl.ds(0, chunks - 1),), misc_sems.at[0])
    read_tail = read(late + (pl.ds(chunks - 1, 1),), misc_sems.at[1])
    read_dw = pltpu.make_async_copy(dw_hbm, dw_ref, misc_sems.at[2])
    read_pw = pltpu.make_async_copy(pw_hbm, pw_ref, misc_sems.at[3])

    read_pw.start()
    read_dw.start()

    @pl.loop(0, early_steps)
    def _(u):
        read(step_index(u), step_sems.at[u]).start()

    read_late.start()
    read_tail.start()
    read_pw.wait()
    read_dw.wait()

    @pl.loop(0, steps)
    def _(u):
        @pl.when(u < early_steps)
        def _():
            read(step_index(u), step_sems.at[u]).wait()

        @pl.when(u == early_steps)
        def _():
            read_late.wait()

        @pl.when(u >= early_steps)
        def _():
            first = 2 * (u - early_steps)
            start_writes(first * _STEP, jnp.minimum(first + 2, u) * _STEP)

        @pl.when(u == early_steps)
        def _():
            read_tail.wait()

        index = step_index(u)
        xv = buf[index].reshape(streams * _STEP * chunk_rows, C)
        scaled = xv.astype(jnp.float32) * dw_ref[0].astype(jnp.float32)
        y = jnp.dot(scaled.astype(xv.dtype), pw_ref[...],
                    preferred_element_type=jnp.float32)
        buf[index] = y.astype(buf.dtype).reshape(streams, _STEP, chunk_rows, C)

    start_writes((steps - 1) * _STEP, steps * _STEP)
    pltpu.make_async_copy(buf, o_hbm, write_sem).wait()


@jax.jit
def pallas_standalone__depthwise_separable__vision_kernel(
    x: jax.Array,
    dw: jax.Array,
    pw: jax.Array,
):
    B, H, W, C = x.shape
    assert dw.shape == (1, 1, C) and pw.shape == (C, C)
    blocks, rest = divmod(B * H * W, _STREAMS * _CHUNKS * _CHUNK_ROWS)
    assert rest == 0 and blocks % 2 == 0
    view = (blocks, _STREAMS, _CHUNKS, _CHUNK_ROWS, C)
    hbm = pl.BlockSpec(memory_space=pltpu.HBM)

    out = pl.pallas_call(
        _kernel,
        in_specs=[hbm, hbm, hbm],
        out_specs=hbm,
        out_shape=jax.ShapeDtypeStruct(view, x.dtype),
        scratch_shapes=[
            pltpu.VMEM(view, x.dtype),
            pltpu.VMEM(dw.shape, dw.dtype),
            pltpu.VMEM(pw.shape, pw.dtype),
            pltpu.SemaphoreType.DMA((blocks // 2 * (_CHUNKS // _STEP),)),
            pltpu.SemaphoreType.DMA((4,)),
            pltpu.SemaphoreType.DMA,
        ],
        compiler_params=pltpu.CompilerParams(vmem_limit_bytes=_VMEM_LIMIT),
    )(x.reshape(view), dw, pw)
    return out.reshape(B, H, W, C)
```
